```python
import jax
import jax.numpy as jnp

def _softmax(x, axis=-1):
    return jax.nn.softmax(x, axis=axis)
def _gelu(x):
    return jax.nn.gelu(x, approximate=True)
def _silu(x):
    return jax.nn.silu(x)
def _sigmoid(x):
    return jax.nn.sigmoid(x)
def _layernorm(x, axis=-1, eps=1e-5):
    m = jnp.mean(x, axis=axis, keepdims=True)
    v = jnp.var(x, axis=axis, keepdims=True)
    return (x - m) / jnp.sqrt(v + eps)
def _scatter_add(tgt, idx, src, axis=0):
    return tgt.at[idx].add(src)
def _segment_sum(src, seg, n):
    return jax.ops.segment_sum(src, seg, n)
class _Rng:
    def __init__(self, key):
        self._k = key
    def _next(self):
        self._k, sub = jax.random.split(self._k)
        return sub
    def normal(self, shape):
        return jax.random.normal(self._next(), shape, dtype=jnp.bfloat16)
    def randint(self, lo, hi, shape):
        return jax.random.randint(self._next(), shape, lo, hi, dtype=jnp.int32)
    def uniform(self, shape, lo=0.0, hi=1.0):
        return jax.random.uniform(self._next(), shape, jnp.bfloat16, lo, hi)
    def permutation(self, n):
        return jax.random.permutation(self._next(), n)


kernel_name = 'recurrent_scan__sliding_block_cached__mixer_s_mlp__decode'

def setup_inputs():
    _rng = _Rng(jax.random.key(int.from_bytes(__import__("os").urandom(4), "little")))
    _w = (lambda a: (lambda t: t.astype(jnp.bfloat16) if jnp.issubdtype(t.dtype, jnp.floating) else t)(jnp.asarray(a)))
    def _A_setup():
        B, Sq, D = 1, 1, 512
        Hq, Hkv, Sk, Dh = 32, 32, 32768, 128
        assert Hq % Hkv == 0, (Hq, Hkv)
        return {
            "x": _w((lambda *s: _rng.normal(s) * 0.05)(B, Sq, D)),
            "k_cache": _w((lambda *s: _rng.normal(s) * 0.05)(B, Hkv, Sk, Dh)),
            "v_cache": _w((lambda *s: _rng.normal(s) * 0.05)(B, Hkv, Sk, Dh)),
            "wq": _w((lambda *s: _rng.normal(s) * 0.05)(D, Hq * Dh) * (D ** -0.5)),
            "wo": _w((lambda *s: _rng.normal(s) * 0.05)(Hq * Dh, D) * ((Hq * Dh) ** -0.5)),
        }
    _A_in = _A_setup()

    def _B_setup():
        B, S, D, F = 1, 1, 512, 1376
        return {
            "x":  _w((lambda *s: _rng.normal(s) * 0.05)(B, S, D)),
            "w1": _w((lambda *s: _rng.normal(s) * 0.05)(D, D) * (D ** -0.5)),
            "w2": _w((lambda *s: _rng.normal(s) * 0.05)(D, D) * (D ** -0.5)),
            "w3": _w((lambda *s: _rng.normal(s) * 0.05)(D, F) * (D ** -0.5)),
            "w4": _w((lambda *s: _rng.normal(s) * 0.05)(F, D) * (F ** -0.5)),
        }
    _B_in = _B_setup()

    return {
        "A_x": _A_in["x"],
        "A_k_cache": _A_in["k_cache"],
        "A_v_cache": _A_in["v_cache"],
        "A_wq": _A_in["wq"],
        "A_wo": _A_in["wo"],
        "B_x": _B_in["x"],
        "B_w1": _B_in["w1"],
        "B_w2": _B_in["w2"],
        "B_w3": _B_in["w3"],
        "B_w4": _B_in["w4"],
    }

def reference(A_x, A_k_cache, A_v_cache, A_wq, A_wo, B_x, B_w1, B_w2, B_w3, B_w4):
    def _A_ref(x, k_cache, v_cache, wq, wo):
        B, Sq, D = x.shape
        Hq, Dh = 32, 128
        Hkv, Sk = k_cache.shape[1], k_cache.shape[2]
        W = min(4096, max(256, Sk // 4))
        rep = Hq // Hkv
        q = (lambda x, *d: x.transpose(*d))((x @ wq).reshape(B, Sq, Hq, Dh), 0, 2, 1, 3)
        k = jnp.repeat(k_cache[:, :, Sk - W:, :], rep, axis=1)
        v = jnp.repeat(v_cache[:, :, Sk - W:, :], rep, axis=1)
        scores = jnp.einsum("bhqd,bhkd->bhqk", q, k) * (Dh ** -0.5)
        p = _softmax(scores, axis=-1)
        o = jnp.einsum("bhqk,bhkd->bhqd", p, v)
        return (lambda x, *d: x.transpose(*d))(o, 0, 2, 1, 3).reshape(B, Sq, Hq * Dh) @ wo

    def _B_ref(x, w1, w2, w3, w4):
        B, S, D = x.shape
        h = _gelu(_layernorm(x, axis=-1) @ w1)
        c = D // 4
        g0 = jnp.pad(h[:, :, 0*c:1*c], ((0, 0), (1, 0), (0, 0)))[:, :S, :]
        g1 = jnp.pad(h[:, :, 1*c:2*c], ((0, 0), (0, 1), (0, 0)))[:, 1:, :]
        g2 = jnp.pad(h[:, :, 2*c:3*c], ((0, 0), (2, 0), (0, 0)))[:, :S, :]
        g3 = jnp.pad(h[:, :, 3*c:   ], ((0, 0), (0, 2), (0, 0)))[:, 2:, :]
        hs = jnp.concatenate([g0, g1, g2, g3], axis=-1) @ w2
        x1 = x + hs
        h2 = _gelu(_layernorm(x1, axis=-1) @ w3) @ w4
        return x1 + h2

    x = A_x
    xn = _layernorm(x, axis=-1)
    s = _A_ref(xn, A_k_cache, A_v_cache, A_wq, A_wo)
    g = _silu(_B_ref(xn, B_w1, B_w2, B_w3, B_w4))
    return x + s * g
```

```python
import functools
import os

import jax
import jax.numpy as jnp
from jax import lax
import jax.experimental.pallas as pl
import jax.experimental.pallas.tpu as pltpu

def _p(name, default):
    return type(default)(os.environ.get("KP_" + name, default))

H = 32
DH = 128
G = 4
NG = H // G
EPS = 1e-5
R = _p("R", 512)
DR = _p("DR", 32)
DK = _p("DK", 2)
NVS = 16
NFILL = _p("NFILL", 86)
P_MLP1 = _p("P_MLP1", 48)
P_MLP2 = _p("P_MLP2", 96)
NOCOMP = _p("NOCOMP", 0)
SCOPES = _p("SCOPES", 0)
WR = 32


def _layernorm(x):
    m = jnp.mean(x, axis=-1, keepdims=True)
    xc = x - m
    v = jnp.mean(xc * xc, axis=-1, keepdims=True)
    return xc / jnp.sqrt(v + EPS)


def _gelu_tanh(x):
    c = 0.7978845608028654
    return 0.5 * x * (1.0 + jnp.tanh(c * (x + 0.044715 * (x * x * x))))


class _nullctx:
    def __enter__(self): return self
    def __exit__(self, *a): return False

def scope(name):
    return jax.named_scope(name) if SCOPES else _nullctx()


def _kernel(x_hbm, k_hbm, v_hbm, wq_hbm, wo_hbm, w3_hbm, w4_hbm, o_ref,
            x_buf, k_buf, v_buf, wq_buf, wo_buf, w3_buf, w4_buf,
            q_scr, s_scr, p_scr, l_scr, acc_scr, out_scr, y_scr, h_scr, g_scr,
            sem_k, sem_v, sem_o, sem_m, *, sk, win):
    start = sk - win
    NC = win // R
    ND = R // DR
    NT = NG * NC
    d = x_buf.shape[-1]
    f = w3_buf.shape[0]
    wo_rows = G * DH
    n_wo = wo_rows // WR

    def k_desc(t, j):
        g = t // NC
        c = t % NC
        return pltpu.make_async_copy(
            k_hbm.at[0, pl.ds(g * G, G), pl.ds(start + c * R + j * DR, DR), :],
            k_buf.at[c, :, pl.ds(j * DR, DR), :], sem_k.at[c])

    def v_desc(t, j):
        g = t // NC
        c = t % NC
        s = t % NVS
        return pltpu.make_async_copy(
            v_hbm.at[0, pl.ds(g * G, G), pl.ds(start + c * R + j * DR, DR), :],
            v_buf.at[s, :, pl.ds(j * DR, DR), :], sem_v.at[s])

    def kv_start(t):
        for j in range(ND):
            k_desc(t, j).start(priority=0)
            v_desc(t, j).start(priority=1)

    def kv_wait(dst, sem, c):
        pltpu.make_async_copy(dst.at[c], dst.at[c], sem.at[c]).wait()

    def wo_wait(g):
        blk = wo_buf.at[pl.ds(g * wo_rows, wo_rows), :]
        pltpu.make_async_copy(blk, blk, sem_o.at[g]).wait()

    def wq_desc(i):
        r0 = (i // 2) * 8
        c0 = (i % 2) * (H * DH // 2)
        return pltpu.make_async_copy(wq_hbm.at[pl.ds(r0, 8), pl.ds(c0, H * DH // 2)],
                                     wq_buf.at[pl.ds(r0, 8), pl.ds(c0, H * DH // 2)], sem_m.at[1])
    n_wq = 2 * d // 8

    def row_desc(src, dst, sem, r):
        return pltpu.make_async_copy(src.at[pl.ds(r, WR), :], dst.at[pl.ds(r, WR), :], sem)

    t1_items = ([row_desc(w3_hbm, w3_buf, sem_m.at[2], r) for r in range(0, f, WR)]
                + [row_desc(w4_hbm, w4_buf, sem_m.at[3], r) for r in range(0, f, WR)]
                + [row_desc(wo_hbm, wo_buf, sem_o.at[r // wo_rows], r) for r in range(0, H * DH, WR)])
    t0_items = [wq_desc(i) for i in range(n_wq)]

    def mlp1():
        pltpu.make_async_copy(w3_buf, w3_buf, sem_m.at[2]).wait()
        if not NOCOMP:
            hmid = lax.dot_general(y_scr[...], w3_buf[...], (((1,), (1,)), ((), ())), preferred_element_type=jnp.float32)
            h_scr[...] = _gelu_tanh(hmid).astype(jnp.bfloat16)

    def mlp2():
        pltpu.make_async_copy(w4_buf, w4_buf, sem_m.at[3]).wait()
        if not NOCOMP:
            h2 = jnp.dot(h_scr[...], w4_buf[...], preferred_element_type=jnp.float32)
            b = xn_r + h2
            g_scr[...] = b * jax.nn.sigmoid(b)

    with scope("pro_issue"):
        x_cp = pltpu.make_async_copy(x_hbm, x_buf, sem_m.at[0])
        x_cp.start(priority=0)
        for it in t1_items[:NFILL]:
            it.start(priority=1)
        rest1 = t1_items[NFILL:]

    with scope("ln"):
        x_cp.wait()
        x = x_buf[0].astype(jnp.float32)
        xn = _layernorm(x)
        xn_b = jnp.broadcast_to(xn, (8, d)).astype(jnp.bfloat16)
        xn_r = xn_b.astype(jnp.float32)
        y_scr[...] = _layernorm(xn_r).astype(jnp.bfloat16)
        acc_scr[...] = jnp.zeros_like(acc_scr)
        out_scr[...] = jnp.zeros_like(out_scr)

    def pairs(lo, hi):
        for i in range(lo, hi):
            if i < len(t0_items): t0_items[i].start(priority=0)
            if i < len(rest1): rest1[i].start(priority=1)

    with scope("pro_issue2"):
        pairs(0, P_MLP1)
    with scope("mlp1"):
        mlp1()
    with scope("pro_issue3"):
        pairs(P_MLP1, P_MLP2)
    with scope("mlp2"):
        mlp2()
    with scope("pro_issue4"):
        pairs(P_MLP2, max(len(t0_items), len(rest1)))
        for t in range(DK):
            kv_start(t)

    with scope("qproj"):
        pltpu.make_async_copy(wq_buf, wq_buf, sem_m.at[1]).wait()
        if not NOCOMP:
            q_all = jnp.dot(xn_b, wq_buf[...], preferred_element_type=jnp.float32).astype(jnp.bfloat16)
            for h in range(H):
                q_scr[h] = q_all[:, h * DH:(h + 1) * DH]

    scale = DH ** -0.5
    row = lax.broadcasted_iota(jnp.int32, (8, R), 0)
    row_d = lax.broadcasted_iota(jnp.int32, (8, DH), 0)

    def qk(t):
        g = t // NC
        c = t % NC
        s = None
        for j in range(G):
            sj = lax.dot_general(q_scr[g * G + j], k_buf[c, j], (((1,), (1,)), ((), ())),
                                 preferred_element_type=jnp.float32)
            s = sj if s is None else jnp.where(row == j, sj, s)
        s_scr[c] = s

    def softmax():
        s = s_scr[...]
        m = jnp.max(jnp.max(s, axis=0), axis=-1, keepdims=True)
        p = jnp.exp((s - m[None]) * scale)
        l_scr[...] = jnp.broadcast_to(jnp.sum(jnp.sum(p, axis=0), axis=-1, keepdims=True), l_scr.shape)
        p_scr[...] = p.astype(jnp.bfloat16)

    def pv(u):
        c = u % NC
        p = p_scr[c]
        o = None
        for j in range(G):
            oj = jnp.dot(p, v_buf[u % NVS, j], preferred_element_type=jnp.float32)
            o = oj if o is None else jnp.where(row_d == j, oj, o)
        acc_scr[...] += o

    def finalize(g, l):
        o = acc_scr[...] / l
        acc_scr[...] = jnp.zeros_like(acc_scr)
        lhs = jnp.concatenate([jnp.where(row_d == j, o, 0.0) for j in range(G)], axis=1).astype(jnp.bfloat16)
        wo_wait(g)
        out_scr[...] += jnp.dot(lhs, wo_buf[pl.ds(pl.multiple_of(g * wo_rows, wo_rows), wo_rows), :],
                                preferred_element_type=jnp.float32)

    NC_LEAD = NC
    n_steps = NT + NC_LEAD

    def step(t, carry):
        with scope("issue"):
            @pl.when(t + DK < NT)
            def _():
                kv_start(t + DK)

        @pl.when(t < NT)
        def _():
            with scope("waitK"):
                kv_wait(k_buf, sem_k, t % NC)
            if not NOCOMP:
                with scope("qk"):
                    qk(t)

        @pl.when(t >= NC_LEAD)
        def _():
            with scope("waitV"):
                kv_wait(v_buf, sem_v, (t - NC_LEAD) % NVS)
            if not NOCOMP:
                with scope("pv"):
                    pv(t - NC_LEAD)

        @pl.when(t % NC == NC - 1)
        def _():
            with scope("fin"):
                @pl.when(t >= NC_LEAD)
                def _():
                    if not NOCOMP:
                        finalize((t - NC_LEAD) // NC, l_scr[...])
                    else:
                        wo_wait((t - NC_LEAD) // NC)
                @pl.when(t < NT)
                def _():
                    if not NOCOMP:
                        softmax()
        return carry

    lax.fori_loop(0, n_steps, step, 0)

    with scope("final"):
        if not NOCOMP:
            attn = jnp.sum(out_scr[...], axis=0, keepdims=True)
            out = x + attn * g_scr[0:1, :]
            o_ref[0] = out.astype(o_ref.dtype)
        else:
            o_ref[0] = x.astype(o_ref.dtype)


@jax.jit
def pallas_recurrent_scan__sliding_block_cached__mixer_s_mlp__decode_kernel(
    A_x, A_k_cache, A_v_cache, A_wq, A_wo, B_x, B_w1, B_w2, B_w3, B_w4,
):
    _, _, d = A_x.shape
    sk = A_k_cache.shape[2]
    win = min(4096, max(256, sk // 4))
    f = B_w3.shape[1]
    bf = jnp.bfloat16
    f32 = jnp.float32
    NC = win // R
    any_spec = pl.BlockSpec(memory_space=pl.ANY)
    return pl.pallas_call(
        functools.partial(_kernel, sk=sk, win=win),
        out_shape=jax.ShapeDtypeStruct(A_x.shape, A_x.dtype),
        in_specs=[any_spec] * 7,
        out_specs=pl.BlockSpec(memory_space=pltpu.VMEM),
        scratch_shapes=[
            pltpu.VMEM(A_x.shape, bf),
            pltpu.VMEM((NC, G, R, DH), bf),
            pltpu.VMEM((NVS, G, R, DH), bf),
            pltpu.VMEM((d, H * DH), bf),
            pltpu.VMEM((H * DH, d), bf),
            pltpu.VMEM((f, d), bf),
            pltpu.VMEM((f, d), bf),
            pltpu.VMEM((H, 8, DH), bf),
            pltpu.VMEM((NC, 8, R), f32),
            pltpu.VMEM((NC, 8, R), bf),
            pltpu.VMEM((8, DH), f32),
            pltpu.VMEM((8, DH), f32),
            pltpu.VMEM((8, d), f32),
            pltpu.VMEM((8, d), bf),
            pltpu.VMEM((8, f), bf),
            pltpu.VMEM((8, d), f32),
            pltpu.SemaphoreType.DMA((NC,)),
            pltpu.SemaphoreType.DMA((NVS,)),
            pltpu.SemaphoreType.DMA((NG,)),
            pltpu.SemaphoreType.DMA((4,)),
        ],
        compiler_params=pltpu.CompilerParams(vmem_limit_bytes=64 * 1024 * 1024,
                                             disable_bounds_checks=bool(_p("NOBC", 1))),
    )(A_x, A_k_cache, A_v_cache, A_wq, A_wo, B_w3.T, B_w4)
```

```python
import functools
import os

import jax
import jax.numpy as jnp
from jax import lax
import jax.experimental.pallas as pl
import jax.experimental.pallas.tpu as pltpu

def _p(name, default):
    return type(default)(os.environ.get("KP_" + name, default))

H = 32
DH = 128
G = 4
NG = H // G
EPS = 1e-5
R = _p("R", 512)
DR = _p("DR", 32)
DK = _p("DK", 3)
LAG = _p("LAG", 3)
NVS = 16
NOCOMP = _p("NOCOMP", 0)
SCOPES = _p("SCOPES", 0)
T_MLP2 = _p("T_MLP2", 2)
WR = 32


def _layernorm(x):
    m = jnp.mean(x, axis=-1, keepdims=True)
    xc = x - m
    v = jnp.mean(xc * xc, axis=-1, keepdims=True)
    return xc / jnp.sqrt(v + EPS)


def _gelu_tanh(x):
    c = 0.7978845608028654
    return 0.5 * x * (1.0 + jnp.tanh(c * (x + 0.044715 * (x * x * x))))


def _div(a, n):
    if isinstance(a, int):
        return a // n
    assert n & (n - 1) == 0
    return lax.shift_right_logical(a, n.bit_length() - 1)


def _mod(a, n):
    if isinstance(a, int):
        return a % n
    assert n & (n - 1) == 0
    return lax.bitwise_and(a, n - 1)


class _nullctx:
    def __enter__(self): return self
    def __exit__(self, *a): return False

def scope(name):
    return jax.named_scope(name) if SCOPES else _nullctx()


def _kernel(x_hbm, k_hbm, v_hbm, wq_hbm, wo_hbm, w3_hbm, w4_hbm, o_ref,
            x_buf, k_buf, v_buf, wq_buf, wo_buf, w3_buf, w4_buf,
            q_scr, s_scr, p_scr, l_scr, acc_scr, out_scr, y_scr, h_scr, g_scr, xn_scr,
            sem_k, sem_v, sem_o, sem_m, *, sk, win):
    start = sk - win
    NC = win // R
    ND = R // DR
    NT = NG * NC
    d = x_buf.shape[-1]
    f = w3_buf.shape[0]
    wo_rows = G * DH
    n_wo_g = wo_rows // WR
    n_wo = H * DH // WR
    n_w3 = f // WR
    n_wq = 2 * d // 8
    half = H * DH // 2

    def k_desc(t, j):
        g = _div(t, NC)
        c = _mod(t, NC)
        return pltpu.make_async_copy(
            k_hbm.at[0, pl.ds(g * G, G), pl.ds(start + c * R + j * DR, DR), :],
            k_buf.at[c, :, pl.ds(j * DR, DR), :], sem_k.at[c])

    def v_desc(t, j):
        g = _div(t, NC)
        c = _mod(t, NC)
        s = _mod(t, NVS)
        return pltpu.make_async_copy(
            v_hbm.at[0, pl.ds(g * G, G), pl.ds(start + c * R + j * DR, DR), :],
            v_buf.at[s, :, pl.ds(j * DR, DR), :], sem_v.at[s])

    def kv_wait(dst, sem, c):
        pltpu.make_async_copy(dst.at[c], dst.at[c], sem.at[c]).wait()

    def wo_wait(g):
        blk = wo_buf.at[pl.ds(g * wo_rows, wo_rows), :]
        pltpu.make_async_copy(blk, blk, sem_o.at[g]).wait()

    def wq_desc(i):
        r0 = pl.multiple_of(_div(i, 2) * 8, 8)
        c0 = pl.multiple_of(_mod(i, 2) * half, half)
        return pltpu.make_async_copy(wq_hbm.at[pl.ds(r0, 8), pl.ds(c0, half)],
                                     wq_buf.at[pl.ds(r0, 8), pl.ds(c0, half)], sem_m.at[1])

    def row_desc(src, dst, sem, i):
        r = pl.multiple_of(i * WR, WR)
        return pltpu.make_async_copy(src.at[pl.ds(r, WR), :], dst.at[pl.ds(r, WR), :], sem)

    def wo_desc(i):
        return row_desc(wo_hbm, wo_buf, sem_o.at[_div(i, n_wo_g)], i)

    def loop(lo, hi, fn):
        def body(i, c):
            fn(i)
            return c
        lax.fori_loop(lo, hi, body, 0)

    def mlp1():
        pltpu.make_async_copy(w3_buf, w3_buf, sem_m.at[2]).wait()
        if not NOCOMP:
            hmid = lax.dot_general(y_scr[...], w3_buf[...], (((1,), (1,)), ((), ())), preferred_element_type=jnp.float32)
            h_scr[...] = _gelu_tanh(hmid).astype(jnp.bfloat16)

    def mlp2():
        pltpu.make_async_copy(w4_buf, w4_buf, sem_m.at[3]).wait()
        if not NOCOMP:
            h2 = jnp.dot(h_scr[...], w4_buf[...], preferred_element_type=jnp.float32)
            b = xn_scr[...].astype(jnp.float32) + h2
            g_scr[...] = b * jax.nn.sigmoid(b)

    x_cp = pltpu.make_async_copy(x_hbm, x_buf, sem_m.at[0])
    with scope("pro_issueA"):
        x_cp.start(priority=0)
        def a1(i):
            wq_desc(i).start(priority=0)
            row_desc(w3_hbm, w3_buf, sem_m.at[2], i).start(priority=1)
        loop(0, n_w3, a1)

    with scope("ln"):
        x_cp.wait()
        x = x_buf[0].astype(jnp.float32)
        xn = _layernorm(x)
        xn_b = jnp.broadcast_to(xn, (8, d)).astype(jnp.bfloat16)
        xn_scr[...] = xn_b
        y_scr[...] = _layernorm(xn_b.astype(jnp.float32)).astype(jnp.bfloat16)
        acc_scr[...] = jnp.zeros_like(acc_scr)
        out_scr[...] = jnp.zeros_like(out_scr)

    n_wo_a = n_wq - n_w3
    with scope("pro_issueA2"):
        def a2(i):
            wq_desc(i).start(priority=0)
            wo_desc(i - n_w3).start(priority=1)
        loop(n_w3, n_wq, a2)

    with scope("mlp1"):
        mlp1()

    n_b = n_wo - n_wo_a
    assert n_b <= LAG * ND <= DK * ND + n_b
    with scope("pro_issueB"):
        def b1(i):
            k_desc(_div(i, ND), _mod(i, ND)).start(priority=0)
            wo_desc(n_wo_a + i).start(priority=1)
        loop(0, n_b, b1)
        def b2(i):
            k_desc(_div(i, ND), _mod(i, ND)).start(priority=0)
        loop(n_b, LAG * ND, b2)
        for t in range(LAG, DK):
            for j in range(ND):
                k_desc(t, j).start(priority=0)
                v_desc(t - LAG, j).start(priority=1)

    with scope("qproj"):
        pltpu.make_async_copy(wq_buf, wq_buf, sem_m.at[1]).wait()
        if not NOCOMP:
            q_all = jnp.dot(xn_scr[...], wq_buf[...], preferred_element_type=jnp.float32).astype(jnp.bfloat16)
            for h in range(H):
                q_scr[h] = q_all[:, h * DH:(h + 1) * DH]

    scale = DH ** -0.5
    row = lax.broadcasted_iota(jnp.int32, (8, R), 0)
    row_d = lax.broadcasted_iota(jnp.int32, (8, DH), 0)

    def qk(t):
        g = _div(t, NC)
        c = _mod(t, NC)
        s = None
        for j in range(G):
            sj = lax.dot_general(q_scr[g * G + j], k_buf[c, j], (((1,), (1,)), ((), ())),
                                 preferred_element_type=jnp.float32)
            s = sj if s is None else jnp.where(row == j, sj, s)
        s_scr[c] = s

    def softmax():
        s = s_scr[...]
        m = jnp.max(jnp.max(s, axis=0), axis=-1, keepdims=True)
        p = jnp.exp((s - m[None]) * scale)
        l_scr[...] = jnp.broadcast_to(jnp.sum(jnp.sum(p, axis=0), axis=-1, keepdims=True), l_scr.shape)
        p_scr[...] = p.astype(jnp.bfloat16)

    def pv(u):
        c = _mod(u, NC)
        p = p_scr[c]
        o = None
        for j in range(G):
            oj = jnp.dot(p, v_buf[_mod(u, NVS), j], preferred_element_type=jnp.float32)
            o = oj if o is None else jnp.where(row_d == j, oj, o)
        acc_scr[...] += o

    def finalize(g, l):
        o = acc_scr[...] / l
        acc_scr[...] = jnp.zeros_like(acc_scr)
        lhs = jnp.concatenate([jnp.where(row_d == j, o, 0.0) for j in range(G)], axis=1).astype(jnp.bfloat16)
        wo_wait(g)
        out_scr[...] += jnp.dot(lhs, wo_buf[pl.ds(pl.multiple_of(g * wo_rows, wo_rows), wo_rows), :],
                                preferred_element_type=jnp.float32)

    NC_LEAD = NC
    n_steps = NT + NC_LEAD
    n_x = -(-n_w3 // ND)

    def step(t, carry):
        with scope("issue"):
            tk = t + DK
            @pl.when(tk < NT)
            def _():
                for j in range(ND):
                    k_desc(tk, j).start(priority=0)
                    v_desc(tk - LAG, j).start(priority=1)
            for i in range(LAG):
                @pl.when(tk == NT + i)
                def _(i=i):
                    for j in range(ND):
                        if i * ND + j < n_w3:
                            row_desc(w4_hbm, w4_buf, sem_m.at[3], i * ND + j).start(priority=0)
                        v_desc(NT - LAG + i, j).start(priority=1)

        @pl.when(t < NT)
        def _():
            with scope("waitK"):
                kv_wait(k_buf, sem_k, _mod(t, NC))
            if not NOCOMP:
                with scope("qk"):
                    qk(t)

        @pl.when(t == n_steps - T_MLP2)
        def _():
            with scope("mlp2"):
                mlp2()

        @pl.when(t >= NC_LEAD)
        def _():
            with scope("waitV"):
                kv_wait(v_buf, sem_v, _mod(t - NC_LEAD, NVS))
            if not NOCOMP:
                with scope("pv"):
                    pv(t - NC_LEAD)

        @pl.when(_mod(t, NC) == NC - 1)
        def _():
            with scope("fin"):
                @pl.when(t >= NC_LEAD)
                def _():
                    if not NOCOMP:
                        finalize(_div(t - NC_LEAD, NC), l_scr[...])
                    else:
                        wo_wait(_div(t - NC_LEAD, NC))
                @pl.when(t < NT)
                def _():
                    if not NOCOMP:
                        softmax()
        return carry

    assert n_w3 <= LAG * ND
    lax.fori_loop(0, n_steps, step, 0)

    with scope("final"):
        x = x_buf[0].astype(jnp.float32)
        if not NOCOMP:
            attn = jnp.sum(out_scr[...], axis=0, keepdims=True)
            out = x + attn * g_scr[0:1, :]
            o_ref[0] = out.astype(o_ref.dtype)
        else:
            o_ref[0] = x.astype(o_ref.dtype)


@jax.jit
def pallas_recurrent_scan__sliding_block_cached__mixer_s_mlp__decode_kernel(
    A_x, A_k_cache, A_v_cache, A_wq, A_wo, B_x, B_w1, B_w2, B_w3, B_w4,
):
    _, _, d = A_x.shape
    sk = A_k_cache.shape[2]
    win = min(4096, max(256, sk // 4))
    f = B_w3.shape[1]
    bf = jnp.bfloat16
    f32 = jnp.float32
    NC = win // R
    any_spec = pl.BlockSpec(memory_space=pl.ANY)
    return pl.pallas_call(
        functools.partial(_kernel, sk=sk, win=win),
        out_shape=jax.ShapeDtypeStruct(A_x.shape, A_x.dtype),
        in_specs=[any_spec] * 7,
        out_specs=pl.BlockSpec(memory_space=pltpu.VMEM),
        scratch_shapes=[
            pltpu.VMEM(A_x.shape, bf),
            pltpu.VMEM((NC, G, R, DH), bf),
            pltpu.VMEM((NVS, G, R, DH), bf),
            pltpu.VMEM((d, H * DH), bf),
            pltpu.VMEM((H * DH, d), bf),
            pltpu.VMEM((f, d), bf),
            pltpu.VMEM((f, d), bf),
            pltpu.VMEM((H, 8, DH), bf),
            pltpu.VMEM((NC, 8, R), f32),
            pltpu.VMEM((NC, 8, R), bf),
            pltpu.VMEM((8, DH), f32),
            pltpu.VMEM((8, DH), f32),
            pltpu.VMEM((8, d), f32),
            pltpu.VMEM((8, d), bf),
            pltpu.VMEM((8, f), bf),
            pltpu.VMEM((8, d), f32),
            pltpu.VMEM((8, d), bf),
            pltpu.SemaphoreType.DMA((NC,)),
            pltpu.SemaphoreType.DMA((NVS,)),
            pltpu.SemaphoreType.DMA((NG,)),
            pltpu.SemaphoreType.DMA((4,)),
        ],
        compiler_params=pltpu.CompilerParams(vmem_limit_bytes=64 * 1024 * 1024,
                                             disable_bounds_checks=bool(_p("NOBC", 1)),
                                             disable_semaphore_checks=bool(_p("NOSC", 1))),
    )(A_x, A_k_cache, A_v_cache, A_wq, A_wo, B_w3.T, B_w4)
```

```python
import functools
import os

import jax
import jax.numpy as jnp
from jax import lax
import jax.experimental.pallas as pl
import jax.experimental.pallas.tpu as pltpu

def _p(name, default):
    return type(default)(os.environ.get("KP_" + name, default))

H = 32
DH = 128
G = 4
NG = H // G
EPS = 1e-5
R = _p("R", 512)
DR = _p("DR", 32)
DK = _p("DK", 3)
LAG = _p("LAG", 3)
NVS = 16
NOCOMP = _p("NOCOMP", 0)
SCOPES = _p("SCOPES", 0)
T_MLP2 = _p("T_MLP2", 2)
WR = 32


def _layernorm(x):
    m = jnp.mean(x, axis=-1, keepdims=True)
    xc = x - m
    v = jnp.mean(xc * xc, axis=-1, keepdims=True)
    return xc / jnp.sqrt(v + EPS)


def _gelu_tanh(x):
    c = 0.7978845608028654
    return 0.5 * x * (1.0 + jnp.tanh(c * (x + 0.044715 * (x * x * x))))


def _div(a, n):
    if isinstance(a, int):
        return a // n
    assert n & (n - 1) == 0
    return lax.shift_right_logical(a, n.bit_length() - 1)


def _mod(a, n):
    if isinstance(a, int):
        return a % n
    assert n & (n - 1) == 0
    return lax.bitwise_and(a, n - 1)


class _nullctx:
    def __enter__(self): return self
    def __exit__(self, *a): return False

def scope(name):
    return jax.named_scope(name) if SCOPES else _nullctx()


def _kernel(x_hbm, k_hbm, v_hbm, wq_hbm, wo_hbm, w3_hbm, w4_hbm, o_ref,
            x_buf, k_buf, v_buf, wq_buf, wo_buf, w3_buf, w4_buf,
            q_scr, s_scr, p_scr, acc_scr, out_scr, y_scr, h_scr, g_scr, xn_scr,
            sem_k, sem_v, sem_l, sem_m, *, sk, win):
    start = sk - win
    NC = win // R
    ND = R // DR
    NT = NG * NC
    d = x_buf.shape[-1]
    f = w3_buf.shape[0] * w3_buf.shape[1]
    wo_rows = G * DH
    n_wo = wo_buf.shape[1] // 8
    n_w3 = w3_buf.shape[1] // 16
    QC = 512
    n_qc = H * DH // QC
    n_wq = (wq_buf.shape[1] // 8) * n_qc

    def k_desc(t, j):
        g = _div(t, NC)
        c = _mod(t, NC)
        return pltpu.make_async_copy(
            k_hbm.at[0, pl.ds(g * G, G), pl.ds(start + c * R + j * DR, DR), :],
            k_buf.at[c, :, pl.ds(j * DR, DR), :], sem_k.at[c])

    def v_desc(t, j):
        g = _div(t, NC)
        c = _mod(t, NC)
        s = _mod(t, NVS)
        return pltpu.make_async_copy(
            v_hbm.at[0, pl.ds(g * G, G), pl.ds(start + c * R + j * DR, DR), :],
            v_buf.at[s, :, pl.ds(j * DR, DR), :], sem_v.at[s])

    def kv_wait(dst, sem, c):
        pltpu.make_async_copy(dst.at[c], dst.at[c], sem.at[c]).wait()

    def wq_desc(i):
        r0 = pl.multiple_of(_div(i, n_qc) * 8, 8)
        c0 = pl.multiple_of(_mod(i, n_qc) * QC, QC)
        return pltpu.make_async_copy(wq_hbm.at[:, pl.ds(r0, 8), pl.ds(c0, QC)],
                                     wq_buf.at[:, pl.ds(r0, 8), pl.ds(c0, QC)], sem_m.at[1])

    def row_desc(src, dst, sem, i, rows):
        r = i * rows if isinstance(i, int) else pl.multiple_of(i * rows, rows)
        return pltpu.make_async_copy(src.at[:, pl.ds(r, rows), :], dst.at[:, pl.ds(r, rows), :], sem)

    def wo_desc(i):
        return row_desc(wo_hbm, wo_buf, sem_m.at[4], i, 8)

    def w3_desc(i):
        return row_desc(w3_hbm, w3_buf, sem_m.at[2], i, 16)

    def w4_desc(i):
        return row_desc(w4_hbm, w4_buf, sem_m.at[3], i, 16)

    def vlast_desc(j, i):
        rr = R // 4
        return pltpu.make_async_copy(
            v_hbm.at[0, H - G + j, pl.ds(start + (NC - 1) * R + i * rr, rr), :],
            v_buf.at[(NT - 1) % NVS, j, pl.ds(i * rr, rr), :], sem_l.at[j])

    def loop(lo, hi, fn):
        def body(i, c):
            fn(i)
            return c
        lax.fori_loop(lo, hi, body, 0)

    def mlp1():
        pltpu.make_async_copy(w3_buf, w3_buf, sem_m.at[2]).wait()
        if not NOCOMP:
            hmid = lax.dot_general(y_scr[...], w3_buf[...].reshape(f, d), (((1,), (1,)), ((), ())), preferred_element_type=jnp.float32)
            h_scr[...] = _gelu_tanh(hmid).astype(jnp.bfloat16)

    def mlp2():
        pltpu.make_async_copy(w4_buf, w4_buf, sem_m.at[3]).wait()
        if not NOCOMP:
            h2 = jnp.dot(h_scr[...], w4_buf[...].reshape(f, d), preferred_element_type=jnp.float32)
            b = xn_scr[...].astype(jnp.float32) + h2
            g_scr[...] = b * jax.nn.sigmoid(b)

    x_cp = pltpu.make_async_copy(x_hbm, x_buf, sem_m.at[0])
    with scope("pro_issueA"):
        x_cp.start(priority=0)
        def a1(i):
            wq_desc(i).start(priority=0)
            w3_desc(i).start(priority=1)
        loop(0, n_w3, a1)

    with scope("ln"):
        x_cp.wait()
        x = x_buf[0].astype(jnp.float32)
        xn = _layernorm(x)
        xn_b = jnp.broadcast_to(xn, (8, d)).astype(jnp.bfloat16)
        xn_scr[...] = xn_b
        y_scr[...] = _layernorm(xn_b.astype(jnp.float32)).astype(jnp.bfloat16)
        acc_scr[...] = jnp.zeros_like(acc_scr)
        out_scr[...] = jnp.zeros_like(out_scr)

    n_wo_a = n_wq - n_w3
    with scope("pro_issueA2"):
        def a2(i):
            wq_desc(i).start(priority=0)
            wo_desc(i - n_w3).start(priority=1)
        loop(n_w3, n_wq, a2)

    with scope("mlp1"):
        mlp1()

    n_b = n_wo - n_wo_a
    assert n_b <= LAG * ND <= DK * ND + n_b
    with scope("pro_issueB"):
        def b1(i):
            k_desc(_div(i, ND), _mod(i, ND)).start(priority=0)
            wo_desc(n_wo_a + i).start(priority=1)
        loop(0, n_b, b1)
        def b2(i):
            k_desc(_div(i, ND), _mod(i, ND)).start(priority=0)
        loop(n_b, LAG * ND, b2)
        for t in range(LAG, DK):
            for j in range(ND):
                k_desc(t, j).start(priority=0)
                v_desc(t - LAG, j).start(priority=1)

    with scope("qproj"):
        pltpu.make_async_copy(wq_buf, wq_buf, sem_m.at[1]).wait()
        if not NOCOMP:
            q_all = jnp.dot(xn_scr[...], wq_buf[...].reshape(d, H * DH), preferred_element_type=jnp.float32).astype(jnp.bfloat16)
            for h in range(H):
                q_scr[h] = q_all[:, h * DH:(h + 1) * DH]

    scale = DH ** -0.5
    row = lax.broadcasted_iota(jnp.int32, (8, R), 0)
    row_d = lax.broadcasted_iota(jnp.int32, (8, DH), 0)

    def qk(t):
        g = _div(t, NC)
        c = _mod(t, NC)
        s = None
        for j in range(G):
            sj = lax.dot_general(q_scr[g * G + j], k_buf[c, j], (((1,), (1,)), ((), ())),
                                 preferred_element_type=jnp.float32)
            s = sj if s is None else jnp.where(row == j, sj, s)
        s_scr[c] = s

    def softmax():
        s = s_scr[...]
        m = jnp.max(jnp.max(s, axis=0), axis=-1, keepdims=True)
        p = jnp.exp((s - m[None]) * scale)
        l = jnp.sum(jnp.sum(p, axis=0), axis=-1, keepdims=True)
        p_scr[...] = (p * (1.0 / l)[None]).astype(jnp.bfloat16)

    def pv(u):
        c = _mod(u, NC)
        p = p_scr[c]
        o = None
        for j in range(G):
            oj = jnp.dot(p, v_buf[_mod(u, NVS), j], preferred_element_type=jnp.float32)
            o = oj if o is None else jnp.where(row_d == j, oj, o)
        acc_scr[...] += o

    def wo_block(g):
        per = wo_buf.shape[1] // wo_rows
        r0 = _mod(g, per) * wo_rows
        return wo_buf[_div(g, per), pl.ds(r0 if isinstance(r0, int) else pl.multiple_of(r0, wo_rows), wo_rows), :]

    def finalize(g):
        o = acc_scr[...]
        acc_scr[...] = jnp.zeros_like(acc_scr)
        lhs = jnp.concatenate([jnp.where(row_d == j, o, 0.0) for j in range(G)], axis=1).astype(jnp.bfloat16)
        out_scr[...] += jnp.dot(lhs, wo_block(g), preferred_element_type=jnp.float32)

    NC_LEAD = NC
    n_steps = NT + NC_LEAD
    n_x = -(-n_w3 // ND)

    def step(t, carry):
        with scope("issue"):
            tk = t + DK
            @pl.when(tk < NT)
            def _():
                for j in range(ND):
                    k_desc(tk, j).start(priority=0)
                    v_desc(tk - LAG, j).start(priority=1)
            for i in range(LAG):
                @pl.when(tk == NT + i)
                def _(i=i):
                    for j in range(ND):
                        if i * ND + j < n_w3:
                            w4_desc(i * ND + j).start(priority=0)
                        if i < LAG - 1:
                            v_desc(NT - LAG + i, j).start(priority=1)
                        else:
                            vlast_desc(j // 4, j % 4).start(priority=1)

        @pl.when(t < NT)
        def _():
            with scope("waitK"):
                kv_wait(k_buf, sem_k, _mod(t, NC))
            if not NOCOMP:
                with scope("qk"):
                    qk(t)

        @pl.when(t == n_steps - T_MLP2)
        def _():
            with scope("mlp2"):
                mlp2()

        @pl.when(t >= NC_LEAD)
        def _():
            with scope("waitV"):
                kv_wait(v_buf, sem_v, _mod(t - NC_LEAD, NVS))
            if not NOCOMP:
                with scope("pv"):
                    pv(t - NC_LEAD)

        @pl.when(_mod(t, NC) == NC - 1)
        def _():
            with scope("fin"):
                @pl.when(t == 2 * NC - 1)
                def _():
                    pltpu.make_async_copy(wo_buf, wo_buf, sem_m.at[4]).wait()
                @pl.when(t >= NC_LEAD)
                def _():
                    if not NOCOMP:
                        finalize(_div(t - NC_LEAD, NC))
                @pl.when(t < NT)
                def _():
                    if not NOCOMP:
                        softmax()
        return carry

    assert n_w3 <= LAG * ND
    assert ND == 16
    lax.fori_loop(0, n_steps - 1, step, 0)

    def wo_head(j):
        h = H - G + j
        per = wo_buf.shape[1] // DH
        return wo_buf[h // per, pl.ds((h % per) * DH, DH), :]

    def last_op(j, oj):
        lhs = jnp.where(row_d == j, acc_scr[...] + oj, 0.0).astype(jnp.bfloat16)
        return jnp.dot(lhs, wo_head(j), preferred_element_type=jnp.float32)

    out_acc = None
    prev = None
    for j in range(G):
        with scope("lastwait"):
            blk = v_buf.at[(NT - 1) % NVS, j]
            pltpu.make_async_copy(blk, blk, sem_l.at[j]).wait()
        if not NOCOMP:
            with scope("lastpv"):
                oj = jnp.dot(p_scr[NC - 1], v_buf[(NT - 1) % NVS, j], preferred_element_type=jnp.float32)
                if prev is not None:
                    c = last_op(j - 1, prev)
                    out_acc = (out_scr[...] if out_acc is None else out_acc) + c
                prev = oj
    if not NOCOMP:
        out_acc = out_acc + last_op(G - 1, prev)

    with scope("final"):
        x = x_buf[0].astype(jnp.float32)
        if not NOCOMP:
            attn = jnp.sum(out_acc, axis=0, keepdims=True)
            out = x + attn * g_scr[0:1, :]
            o_ref[0] = out.astype(o_ref.dtype)
        else:
            o_ref[0] = x.astype(o_ref.dtype)


@jax.jit
def pallas_recurrent_scan__sliding_block_cached__mixer_s_mlp__decode_kernel(
    A_x, A_k_cache, A_v_cache, A_wq, A_wo, B_x, B_w1, B_w2, B_w3, B_w4,
):
    _, _, d = A_x.shape
    sk = A_k_cache.shape[2]
    win = min(4096, max(256, sk // 4))
    f = B_w3.shape[1]
    bf = jnp.bfloat16
    f32 = jnp.float32
    NC = win // R
    any_spec = pl.BlockSpec(memory_space=pl.ANY)
    return pl.pallas_call(
        functools.partial(_kernel, sk=sk, win=win),
        out_shape=jax.ShapeDtypeStruct(A_x.shape, A_x.dtype),
        in_specs=[any_spec] * 7,
        out_specs=pl.BlockSpec(memory_space=pltpu.VMEM),
        scratch_shapes=[
            pltpu.VMEM(A_x.shape, bf),
            pltpu.VMEM((NC, G, R, DH), bf),
            pltpu.VMEM((NVS, G, R, DH), bf),
            pltpu.VMEM((4, d // 4, H * DH), bf),
            pltpu.VMEM((4, H * DH // 4, d), bf),
            pltpu.VMEM((2, f // 2, d), bf),
            pltpu.VMEM((2, f // 2, d), bf),
            pltpu.VMEM((H, 8, DH), bf),
            pltpu.VMEM((NC, 8, R), f32),
            pltpu.VMEM((NC, 8, R), bf),
            pltpu.VMEM((8, DH), f32),
            pltpu.VMEM((8, d), f32),
            pltpu.VMEM((8, d), bf),
            pltpu.VMEM((8, f), bf),
            pltpu.VMEM((8, d), f32),
            pltpu.VMEM((8, d), bf),
            pltpu.SemaphoreType.DMA((NC,)),
            pltpu.SemaphoreType.DMA((NVS,)),
            pltpu.SemaphoreType.DMA((G,)),
            pltpu.SemaphoreType.DMA((5,)),
        ],
        compiler_params=pltpu.CompilerParams(vmem_limit_bytes=64 * 1024 * 1024,
                                             disable_bounds_checks=bool(_p("NOBC", 1)),
                                             disable_semaphore_checks=bool(_p("NOSC", 1))),
    )(A_x, A_k_cache, A_v_cache, A_wq.reshape(4, d // 4, H * DH), A_wo.reshape(4, H * DH // 4, d),
      B_w3.T.reshape(2, f // 2, d), B_w4.reshape(2, f // 2, d))
```

```python
import functools

import jax
import jax.numpy as jnp
from jax import lax
import jax.experimental.pallas as pl
import jax.experimental.pallas.tpu as pltpu

H = 32
DH = 128
G = 4
NG = H // G
EPS = 1e-5
R = 512
DR = 32
DK = 3
LAG = 3
NVS = 16
QC = 512
N_LAST = 4


def _layernorm(x):
    m = jnp.mean(x, axis=-1, keepdims=True)
    xc = x - m
    v = jnp.mean(xc * xc, axis=-1, keepdims=True)
    return xc / jnp.sqrt(v + EPS)


def _gelu_tanh(x):
    c = 0.7978845608028654
    return 0.5 * x * (1.0 + jnp.tanh(c * (x + 0.044715 * (x * x * x))))


def _div(a, n):
    if isinstance(a, int):
        return a // n
    assert n & (n - 1) == 0
    return lax.shift_right_logical(a, n.bit_length() - 1)


def _mod(a, n):
    if isinstance(a, int):
        return a % n
    assert n & (n - 1) == 0
    return lax.bitwise_and(a, n - 1)


def _aligned(i, n):
    return i * n if isinstance(i, int) else pl.multiple_of(i * n, n)


def _wait_all(blk, sem):
    pltpu.make_async_copy(blk, blk, sem).wait()


def _loop(lo, hi, fn):
    def body(i, c):
        fn(i)
        return c
    lax.fori_loop(lo, hi, body, 0)


def _kernel(x_hbm, k_hbm, v_hbm, wq_hbm, wo_hbm, w3_hbm, w4_hbm, o_ref,
            x_buf, k_buf, v_buf, wq_buf, wo_buf, w3_buf, w4_buf,
            q_scr, s_scr, p_scr, acc_scr, out_scr, y_scr, h_scr, g_scr, xn_scr,
            sem_k, sem_v, sem_l, sem_m, *, sk, win):
    start = sk - win
    nc = win // R
    nd = R // DR
    nt = NG * nc
    d = x_buf.shape[-1]
    f = w3_buf.shape[0] * w3_buf.shape[1]
    wo_rows = G * DH
    n_rb = wo_rows // 8
    n_w3 = w3_buf.shape[1] // 16
    n_qc = H * DH // QC
    n_wq = (wq_buf.shape[1] // 8) * n_qc
    n_wl = wo_rows // 32
    s_x, s_wq, s_w3, s_w4, s_wo, s_wol = (sem_m.at[i] for i in range(6))
    last_slot = (nt - 1) % NVS

    def k_desc(t, j):
        g, c = _div(t, nc), _mod(t, nc)
        return pltpu.make_async_copy(
            k_hbm.at[0, pl.ds(g * G, G), pl.ds(start + c * R + j * DR, DR), :],
            k_buf.at[c, :, pl.ds(j * DR, DR), :], sem_k.at[c])

    def v_desc(t, j):
        g, c, s = _div(t, nc), _mod(t, nc), _mod(t, NVS)
        return pltpu.make_async_copy(
            v_hbm.at[0, pl.ds(g * G, G), pl.ds(start + c * R + j * DR, DR), :],
            v_buf.at[s, :, pl.ds(j * DR, DR), :], sem_v.at[s])

    def v_last_desc(j, i):
        rr = R // 4
        return pltpu.make_async_copy(
            v_hbm.at[0, H - G + j, pl.ds(start + (nc - 1) * R + i * rr, rr), :],
            v_buf.at[last_slot, j, pl.ds(i * rr, rr), :], sem_l.at[j])

    def wq_desc(i):
        rows = pl.ds(_aligned(_div(i, n_qc), 8), 8)
        cols = pl.ds(_aligned(_mod(i, n_qc), QC), QC)
        return pltpu.make_async_copy(wq_hbm.at[:, rows, cols], wq_buf.at[:, rows, cols], s_wq)

    def wo_desc(g0, ng, i):
        idx = (pl.ds(g0, ng), pl.ds(_aligned(i, 8), 8), slice(None))
        return pltpu.make_async_copy(wo_hbm.at[idx], wo_buf.at[idx], s_wo)

    def wo_last_desc(i, sem):
        idx = (NG - 1, pl.ds(_aligned(i, 32), 32), slice(None))
        return pltpu.make_async_copy(wo_hbm.at[idx], wo_buf.at[idx], sem)

    def mlp_desc(src, dst, sem, i):
        idx = (slice(None), pl.ds(_aligned(i, 16), 16), slice(None))
        return pltpu.make_async_copy(src.at[idx], dst.at[idx], sem)

    x_cp = pltpu.make_async_copy(x_hbm, x_buf, s_x)
    x_cp.start(priority=0)

    def pair_wq_w3(i):
        wq_desc(i).start(priority=0)
        mlp_desc(w3_hbm, w3_buf, s_w3, i).start(priority=1)
    _loop(0, n_w3, pair_wq_w3)

    x_cp.wait()
    xn_b = jnp.broadcast_to(_layernorm(x_buf[0].astype(jnp.float32)), (8, d)).astype(jnp.bfloat16)
    xn_scr[...] = xn_b
    y_scr[...] = _layernorm(xn_b.astype(jnp.float32)).astype(jnp.bfloat16)
    acc_scr[...] = jnp.zeros_like(acc_scr)
    out_scr[...] = jnp.zeros_like(out_scr)

    n_b1 = n_wq - n_w3 - n_rb

    def pair_wq_wo_a(i):
        wq_desc(i).start(priority=0)
        wo_desc(0, 4, i - n_w3).start(priority=1)
    _loop(n_w3, n_w3 + n_rb, pair_wq_wo_a)

    def pair_wq_wo_b(i):
        wq_desc(i).start(priority=0)
        wo_desc(4, NG - 1 - 4, i - n_w3 - n_rb).start(priority=1)
    _loop(n_w3 + n_rb, n_wq, pair_wq_wo_b)

    _wait_all(w3_buf, s_w3)
    hmid = lax.dot_general(y_scr[...], w3_buf[...].reshape(f, d), (((1,), (1,)), ((), ())),
                           preferred_element_type=jnp.float32)
    h_scr[...] = _gelu_tanh(hmid).astype(jnp.bfloat16)

    n_b = n_rb - n_b1
    assert n_b <= LAG * nd and DK == LAG

    def pair_k_wo(i):
        k_desc(_div(i, nd), _mod(i, nd)).start(priority=0)
        wo_desc(4, NG - 1 - 4, n_b1 + i).start(priority=1)
    _loop(0, n_b, pair_k_wo)
    _loop(n_b, LAG * nd, lambda i: k_desc(_div(i, nd), _mod(i, nd)).start(priority=0))
    _loop(0, n_wl - N_LAST, lambda i: wo_last_desc(i, s_wol).start(priority=1))

    _wait_all(wq_buf, s_wq)
    q_all = jnp.dot(xn_scr[...], wq_buf[...].reshape(d, H * DH),
                    preferred_element_type=jnp.float32).astype(jnp.bfloat16)
    for h in range(H):
        q_scr[h] = q_all[:, h * DH:(h + 1) * DH]

    scale = DH ** -0.5
    row = lax.broadcasted_iota(jnp.int32, (8, R), 0)
    row_d = lax.broadcasted_iota(jnp.int32, (8, DH), 0)

    def qk(t):
        g, c = _div(t, nc), _mod(t, nc)
        s = None
        for j in range(G):
            sj = lax.dot_general(q_scr[g * G + j], k_buf[c, j], (((1,), (1,)), ((), ())),
                                 preferred_element_type=jnp.float32)
            s = sj if s is None else jnp.where(row == j, sj, s)
        s_scr[c] = s

    def softmax():
        s = s_scr[...]
        m = jnp.max(jnp.max(s, axis=0), axis=-1, keepdims=True)
        p = jnp.exp((s - m[None]) * scale)
        l = jnp.sum(jnp.sum(p, axis=0), axis=-1, keepdims=True)
        p_scr[...] = (p * (1.0 / l)[None]).astype(jnp.bfloat16)

    def pv(u):
        p = p_scr[_mod(u, nc)]
        o = None
        for j in range(G):
            oj = jnp.dot(p, v_buf[_mod(u, NVS), j], preferred_element_type=jnp.float32)
            o = oj if o is None else jnp.where(row_d == j, oj, o)
        acc_scr[...] += o

    def finalize(g):
        o = acc_scr[...]
        acc_scr[...] = jnp.zeros_like(acc_scr)
        lhs = jnp.concatenate([jnp.where(row_d == j, o, 0.0) for j in range(G)],
                              axis=1).astype(jnp.bfloat16)
        out_scr[...] += jnp.dot(lhs, wo_buf[g], preferred_element_type=jnp.float32)

    n_steps = nt + nc
    assert n_w3 <= LAG * nd and nd == 4 * G and n_wl - N_LAST == (G - 1) * DH // 32

    def step(t, carry):
        tk = t + DK

        @pl.when(tk < nt)
        def _():
            for j in range(nd):
                k_desc(tk, j).start(priority=0)
                v_desc(tk - LAG, j).start(priority=1)

        for i in range(LAG):
            @pl.when(tk == nt + i)
            def _(i=i):
                for j in range(nd):
                    if i * nd + j < n_w3:
                        mlp_desc(w4_hbm, w4_buf, s_w4, i * nd + j).start(priority=0)
                    if i < LAG - 1:
                        v_desc(nt - LAG + i, j).start(priority=1)
                    else:
                        v_last_desc(j // 4, j % 4).start(priority=1)
                if i == LAG - 1:
                    for ii in range(n_wl - N_LAST, n_wl):
                        wo_last_desc(ii, sem_l.at[G]).start(priority=1)

        @pl.when(t < nt)
        def _():
            _wait_all(k_buf.at[_mod(t, nc)], sem_k.at[_mod(t, nc)])
            qk(t)

        @pl.when(t == n_steps - 2)
        def _():
            _wait_all(w4_buf, s_w4)
            h2 = jnp.dot(h_scr[...], w4_buf[...].reshape(f, d), preferred_element_type=jnp.float32)
            b = xn_scr[...].astype(jnp.float32) + h2
            g_scr[...] = b * jax.nn.sigmoid(b)

        @pl.when(t >= nc)
        def _():
            s = _mod(t - nc, NVS)
            _wait_all(v_buf.at[s], sem_v.at[s])
            pv(t - nc)

        @pl.when(_mod(t, nc) == nc - 1)
        def _():
            @pl.when(t == 2 * nc - 1)
            def _():
                _wait_all(wo_buf.at[pl.ds(0, NG - 1)], s_wo)
                _wait_all(wo_buf.at[NG - 1, pl.ds(0, (G - 1) * DH), :], s_wol)

            @pl.when(t >= nc)
            def _():
                finalize(_div(t - nc, nc))

            @pl.when(t < nt)
            def _():
                softmax()
        return carry

    lax.fori_loop(0, n_steps - 1, step, 0)

    def last_op(lhs, j):
        return jnp.dot(lhs, wo_buf[NG - 1, pl.ds(j * DH, DH), :], preferred_element_type=jnp.float32)

    out_acc = out_scr[...]
    prev = None
    for j in range(G):
        _wait_all(v_buf.at[last_slot, j], sem_l.at[j])
        oj = jnp.dot(p_scr[nc - 1], v_buf[last_slot, j], preferred_element_type=jnp.float32)
        if prev is not None:
            out_acc = out_acc + last_op(prev, j - 1)
        prev = jnp.where(row_d == j, acc_scr[...] + oj, 0.0).astype(jnp.bfloat16)
    part = jnp.sum(out_acc, axis=0, keepdims=True)
    _wait_all(wo_buf.at[NG - 1, pl.ds((G - 1) * DH, DH), :], sem_l.at[G])
    attn = part + last_op(prev, G - 1)[G - 1:G, :]
    out = x_buf[0].astype(jnp.float32) + attn * g_scr[0:1, :]
    o_ref[0] = out.astype(o_ref.dtype)


@jax.jit
def pallas_recurrent_scan__sliding_block_cached__mixer_s_mlp__decode_kernel(
    A_x: jax.Array,
    A_k_cache: jax.Array,
    A_v_cache: jax.Array,
    A_wq: jax.Array,
    A_wo: jax.Array,
    B_x: jax.Array,
    B_w1: jax.Array,
    B_w2: jax.Array,
    B_w3: jax.Array,
    B_w4: jax.Array,
):
    _, _, d = A_x.shape
    sk = A_k_cache.shape[2]
    win = min(4096, max(256, sk // 4))
    f = B_w3.shape[1]
    bf = jnp.bfloat16
    f32 = jnp.float32
    nc = win // R
    any_spec = pl.BlockSpec(memory_space=pl.ANY)
    return pl.pallas_call(
        functools.partial(_kernel, sk=sk, win=win),
        out_shape=jax.ShapeDtypeStruct(A_x.shape, A_x.dtype),
        in_specs=[any_spec] * 7,
        out_specs=pl.BlockSpec(memory_space=pltpu.VMEM),
        scratch_shapes=[
            pltpu.VMEM(A_x.shape, bf),
            pltpu.VMEM((nc, G, R, DH), bf),
            pltpu.VMEM((NVS, G, R, DH), bf),
            pltpu.VMEM((4, d // 4, H * DH), bf),
            pltpu.VMEM((NG, G * DH, d), bf),
            pltpu.VMEM((2, f // 2, d), bf),
            pltpu.VMEM((2, f // 2, d), bf),
            pltpu.VMEM((H, 8, DH), bf),
            pltpu.VMEM((nc, 8, R), f32),
            pltpu.VMEM((nc, 8, R), bf),
            pltpu.VMEM((8, DH), f32),
            pltpu.VMEM((8, d), f32),
            pltpu.VMEM((8, d), bf),
            pltpu.VMEM((8, f), bf),
            pltpu.VMEM((8, d), f32),
            pltpu.VMEM((8, d), bf),
            pltpu.SemaphoreType.DMA((nc,)),
            pltpu.SemaphoreType.DMA((NVS,)),
            pltpu.SemaphoreType.DMA((G + 1,)),
            pltpu.SemaphoreType.DMA((6,)),
        ],
        compiler_params=pltpu.CompilerParams(
            vmem_limit_bytes=64 * 1024 * 1024,
            disable_bounds_checks=True,
            disable_semaphore_checks=True,
        ),
    )(A_x, A_k_cache, A_v_cache,
      A_wq.reshape(4, d // 4, H * DH), A_wo.reshape(NG, G * DH, d),
      B_w3.T.reshape(2, f // 2, d), B_w4.reshape(2, f // 2, d))
```

```python
import functools

import jax
import jax.numpy as jnp
from jax import lax
import jax.experimental.pallas as pl
import jax.experimental.pallas.tpu as pltpu

H = 32
DH = 128
G = 4
NG = H // G
EPS = 1e-5
R = 512
DR = 32
DK = 3
LAG = 3
NVS = 16
QC = 512
N_LEAD = 32
N_LAST = 4


def _layernorm(x):
    m = jnp.mean(x, axis=-1, keepdims=True)
    xc = x - m
    v = jnp.mean(xc * xc, axis=-1, keepdims=True)
    return xc / jnp.sqrt(v + EPS)


def _gelu_tanh(x):
    c = 0.7978845608028654
    return 0.5 * x * (1.0 + jnp.tanh(c * (x + 0.044715 * (x * x * x))))


def _div(a, n):
    if isinstance(a, int):
        return a // n
    assert n & (n - 1) == 0
    return lax.shift_right_logical(a, n.bit_length() - 1)


def _mod(a, n):
    if isinstance(a, int):
        return a % n
    assert n & (n - 1) == 0
    return lax.bitwise_and(a, n - 1)


def _aligned(i, n):
    return i * n if isinstance(i, int) else pl.multiple_of(i * n, n)


def _wait_all(blk, sem):
    pltpu.make_async_copy(blk, blk, sem).wait()


def _loop(lo, hi, fn):
    def body(i, c):
        fn(i)
        return c
    lax.fori_loop(lo, hi, body, 0)


def _kernel(x_hbm, k_hbm, v_hbm, wq_hbm, wo_hbm, w3_hbm, w4_hbm, o_ref,
            x_buf, k_buf, v_buf, wq_buf, wo_buf, w3_buf, w4_buf,
            q_scr, s_scr, p_scr, acc_scr, out_scr, y_scr, h_scr, g_scr, xn_scr,
            sem_k, sem_v, sem_l, sem_m, *, sk, win):
    start = sk - win
    nc = win // R
    nd = R // DR
    nt = NG * nc
    d = x_buf.shape[-1]
    f = w3_buf.shape[0] * w3_buf.shape[1]
    wo_rows = G * DH
    n_rb = wo_rows // 8
    n_w3 = w3_buf.shape[1] // 16
    n_qc = H * DH // QC
    n_wq = (wq_buf.shape[1] // 8) * n_qc
    n_wl = wo_rows // 32
    s_x, s_wq, s_w3, s_w4, s_wo, s_wol = (sem_m.at[i] for i in range(6))
    last_slot = (nt - 1) % NVS

    def k_desc(t, j):
        g, c = _div(t, nc), _mod(t, nc)
        return pltpu.make_async_copy(
            k_hbm.at[0, pl.ds(g * G, G), pl.ds(start + c * R + j * DR, DR), :],
            k_buf.at[c, :, pl.ds(j * DR, DR), :], sem_k.at[c])

    def v_desc(t, j):
        g, c, s = _div(t, nc), _mod(t, nc), _mod(t, NVS)
        return pltpu.make_async_copy(
            v_hbm.at[0, pl.ds(g * G, G), pl.ds(start + c * R + j * DR, DR), :],
            v_buf.at[s, :, pl.ds(j * DR, DR), :], sem_v.at[s])

    def v_last_desc(j, i):
        rr = R // 4
        return pltpu.make_async_copy(
            v_hbm.at[0, H - G + j, pl.ds(start + (nc - 1) * R + i * rr, rr), :],
            v_buf.at[last_slot, j, pl.ds(i * rr, rr), :], sem_l.at[j])

    def wq_desc(i):
        rows = pl.ds(_aligned(_div(i, n_qc), 8), 8)
        cols = pl.ds(_aligned(_mod(i, n_qc), QC), QC)
        return pltpu.make_async_copy(wq_hbm.at[:, rows, cols], wq_buf.at[:, rows, cols], s_wq)

    def wo_desc(g0, ng, i):
        idx = (pl.ds(g0, ng), pl.ds(_aligned(i, 8), 8), slice(None))
        return pltpu.make_async_copy(wo_hbm.at[idx], wo_buf.at[idx], s_wo)

    def wo_last_desc(i, sem):
        idx = (NG - 1, pl.ds(_aligned(i, 32), 32), slice(None))
        return pltpu.make_async_copy(wo_hbm.at[idx], wo_buf.at[idx], sem)

    def mlp_desc(src, dst, sem, i):
        idx = (slice(None), pl.ds(_aligned(i, 16), 16), slice(None))
        return pltpu.make_async_copy(src.at[idx], dst.at[idx], sem)

    x_cp = pltpu.make_async_copy(x_hbm, x_buf, s_x)
    x_cp.start(priority=0)

    _loop(0, N_LEAD, lambda i: mlp_desc(w3_hbm, w3_buf, s_w3, i).start(priority=1))

    n_q1 = N_LEAD // 2
    n_q0 = n_wq - n_q1
    a1 = n_w3 - N_LEAD
    a2 = a1 + n_q1
    a3 = a2 + n_rb
    n_b1 = n_q0 - a3

    def pairs(lo, hi, second):
        def fn(i):
            wq_desc(i).start(priority=0)
            second(i - lo).start(priority=1)
        _loop(lo, hi, fn)

    pairs(0, a1, lambda i: mlp_desc(w3_hbm, w3_buf, s_w3, N_LEAD + i))
    pairs(a1, a2, lambda i: wq_desc(n_q0 + i))

    x_cp.wait()
    xn_b = jnp.broadcast_to(_layernorm(x_buf[0].astype(jnp.float32)), (8, d)).astype(jnp.bfloat16)
    xn_scr[...] = xn_b
    y_scr[...] = _layernorm(xn_b.astype(jnp.float32)).astype(jnp.bfloat16)
    acc_scr[...] = jnp.zeros_like(acc_scr)
    out_scr[...] = jnp.zeros_like(out_scr)

    pairs(a2, a3, lambda i: wo_desc(0, 4, i))
    pairs(a3, n_q0, lambda i: wo_desc(4, NG - 1 - 4, i))

    _wait_all(w3_buf, s_w3)
    hmid = lax.dot_general(y_scr[...], w3_buf[...].reshape(f, d), (((1,), (1,)), ((), ())),
                           preferred_element_type=jnp.float32)
    h_scr[...] = _gelu_tanh(hmid).astype(jnp.bfloat16)

    n_b = n_rb - n_b1
    assert n_b <= LAG * nd and DK == LAG

    def pair_k_wo(i):
        k_desc(_div(i, nd), _mod(i, nd)).start(priority=0)
        wo_desc(4, NG - 1 - 4, n_b1 + i).start(priority=1)
    _loop(0, n_b, pair_k_wo)

    def pair_k_wol(i):
        k_desc(_div(i, nd), _mod(i, nd)).start(priority=0)
        wo_last_desc(i - n_b, s_wol).start(priority=1)
    _loop(n_b, LAG * nd, pair_k_wol)
    _loop(LAG * nd - n_b, n_wl - N_LAST, lambda i: wo_last_desc(i, s_wol).start(priority=1))

    _wait_all(wq_buf, s_wq)
    q_all = jnp.dot(xn_scr[...], wq_buf[...].reshape(d, H * DH),
                    preferred_element_type=jnp.float32).astype(jnp.bfloat16)
    for h in range(H):
        q_scr[h] = q_all[:, h * DH:(h + 1) * DH]

    scale = DH ** -0.5
    row = lax.broadcasted_iota(jnp.int32, (8, R), 0)
    row_d = lax.broadcasted_iota(jnp.int32, (8, DH), 0)

    def qk(t):
        g, c = _div(t, nc), _mod(t, nc)
        s = None
        for j in range(G):
            sj = lax.dot_general(q_scr[g * G + j], k_buf[c, j], (((1,), (1,)), ((), ())),
                                 preferred_element_type=jnp.float32)
            s = sj if s is None else jnp.where(row == j, sj, s)
        s_scr[c] = s

    def softmax():
        s = s_scr[...]
        m = jnp.max(jnp.max(s, axis=0), axis=-1, keepdims=True)
        p = jnp.exp((s - m[None]) * scale)
        l = jnp.sum(jnp.sum(p, axis=0), axis=-1, keepdims=True)
        p_scr[...] = (p * (1.0 / l)[None]).astype(jnp.bfloat16)

    def pv(u):
        p = p_scr[_mod(u, nc)]
        o = None
        for j in range(G):
            oj = jnp.dot(p, v_buf[_mod(u, NVS), j], preferred_element_type=jnp.float32)
            o = oj if o is None else jnp.where(row_d == j, oj, o)
        acc_scr[...] += o

    def finalize(g):
        o = acc_scr[...]
        acc_scr[...] = jnp.zeros_like(acc_scr)
        lhs = jnp.concatenate([jnp.where(row_d == j, o, 0.0) for j in range(G)],
                              axis=1).astype(jnp.bfloat16)
        out_scr[...] += jnp.dot(lhs, wo_buf[g], preferred_element_type=jnp.float32)

    n_steps = nt + nc
    assert n_w3 <= LAG * nd and nd == 4 * G and n_wl - N_LAST == (G - 1) * DH // 32

    def step(t, carry):
        tk = t + DK

        @pl.when(tk < nt)
        def _():
            for j in range(nd):
                k_desc(tk, j).start(priority=0)
                v_desc(tk - LAG, j).start(priority=1)

        for i in range(LAG):
            @pl.when(tk == nt + i)
            def _(i=i):
                for j in range(nd):
                    if i * nd + j < n_w3:
                        mlp_desc(w4_hbm, w4_buf, s_w4, i * nd + j).start(priority=0)
                    if i < LAG - 1:
                        v_desc(nt - LAG + i, j).start(priority=1)
                    else:
                        v_last_desc(j // 4, j % 4).start(priority=1)
                if i == LAG - 1:
                    for ii in range(n_wl - N_LAST, n_wl):
                        wo_last_desc(ii, sem_l.at[G]).start(priority=1)

        @pl.when(t < nt)
        def _():
            _wait_all(k_buf.at[_mod(t, nc)], sem_k.at[_mod(t, nc)])
            qk(t)

        @pl.when(t == n_steps - 2)
        def _():
            _wait_all(w4_buf, s_w4)
            h2 = jnp.dot(h_scr[...], w4_buf[...].reshape(f, d), preferred_element_type=jnp.float32)
            b = xn_scr[...].astype(jnp.float32) + h2
            g_scr[...] = b * jax.nn.sigmoid(b)

        @pl.when(t >= nc)
        def _():
            s = _mod(t - nc, NVS)
            _wait_all(v_buf.at[s], sem_v.at[s])
            pv(t - nc)

        @pl.when(_mod(t, nc) == nc - 1)
        def _():
            @pl.when(t == 2 * nc - 1)
            def _():
                _wait_all(wo_buf.at[pl.ds(0, NG - 1)], s_wo)
                _wait_all(wo_buf.at[NG - 1, pl.ds(0, (G - 1) * DH), :], s_wol)

            @pl.when(t >= nc)
            def _():
                finalize(_div(t - nc, nc))

            @pl.when(t < nt)
            def _():
                softmax()
        return carry

    lax.fori_loop(0, n_steps - 1, step, 0)

    def last_op(lhs, j):
        return jnp.dot(lhs, wo_buf[NG - 1, pl.ds(j * DH, DH), :], preferred_element_type=jnp.float32)

    out_acc = out_scr[...]
    prev = None
    for j in range(G):
        _wait_all(v_buf.at[last_slot, j], sem_l.at[j])
        oj = jnp.dot(p_scr[nc - 1], v_buf[last_slot, j], preferred_element_type=jnp.float32)
        if prev is not None:
            out_acc = out_acc + last_op(prev, j - 1)
        prev = jnp.where(row_d == j, acc_scr[...] + oj, 0.0).astype(jnp.bfloat16)
    part = jnp.sum(out_acc, axis=0, keepdims=True)
    _wait_all(wo_buf.at[NG - 1, pl.ds((G - 1) * DH, DH), :], sem_l.at[G])
    attn = part + last_op(prev, G - 1)[G - 1:G, :]
    out = x_buf[0].astype(jnp.float32) + attn * g_scr[0:1, :]
    o_ref[0] = out.astype(o_ref.dtype)


@jax.jit
def pallas_recurrent_scan__sliding_block_cached__mixer_s_mlp__decode_kernel(
    A_x: jax.Array,
    A_k_cache: jax.Array,
    A_v_cache: jax.Array,
    A_wq: jax.Array,
    A_wo: jax.Array,
    B_x: jax.Array,
    B_w1: jax.Array,
    B_w2: jax.Array,
    B_w3: jax.Array,
    B_w4: jax.Array,
):
    _, _, d = A_x.shape
    sk = A_k_cache.shape[2]
    win = min(4096, max(256, sk // 4))
    f = B_w3.shape[1]
    bf = jnp.bfloat16
    f32 = jnp.float32
    nc = win // R
    any_spec = pl.BlockSpec(memory_space=pl.ANY)
    return pl.pallas_call(
        functools.partial(_kernel, sk=sk, win=win),
        out_shape=jax.ShapeDtypeStruct(A_x.shape, A_x.dtype),
        in_specs=[any_spec] * 7,
        out_specs=pl.BlockSpec(memory_space=pltpu.VMEM),
        scratch_shapes=[
            pltpu.VMEM(A_x.shape, bf),
            pltpu.VMEM((nc, G, R, DH), bf),
            pltpu.VMEM((NVS, G, R, DH), bf),
            pltpu.VMEM((4, d // 4, H * DH), bf),
            pltpu.VMEM((NG, G * DH, d), bf),
            pltpu.VMEM((2, f // 2, d), bf),
            pltpu.VMEM((2, f // 2, d), bf),
            pltpu.VMEM((H, 8, DH), bf),
            pltpu.VMEM((nc, 8, R), f32),
            pltpu.VMEM((nc, 8, R), bf),
            pltpu.VMEM((8, DH), f32),
            pltpu.VMEM((8, d), f32),
            pltpu.VMEM((8, d), bf),
            pltpu.VMEM((8, f), bf),
            pltpu.VMEM((8, d), f32),
            pltpu.VMEM((8, d), bf),
            pltpu.SemaphoreType.DMA((nc,)),
            pltpu.SemaphoreType.DMA((NVS,)),
            pltpu.SemaphoreType.DMA((G + 1,)),
            pltpu.SemaphoreType.DMA((6,)),
        ],
        compiler_params=pltpu.CompilerParams(
            vmem_limit_bytes=64 * 1024 * 1024,
            disable_bounds_checks=True,
            disable_semaphore_checks=True,
        ),
    )(A_x, A_k_cache, A_v_cache,
      A_wq.reshape(4, d // 4, H * DH), A_wo.reshape(NG, G * DH, d),
      B_w3.T.reshape(2, f // 2, d), B_w4.reshape(2, f // 2, d))
```

```python
import functools

import jax
import jax.numpy as jnp
from jax import lax
import jax.experimental.pallas as pl
import jax.experimental.pallas.tpu as pltpu

H = 32
DH = 128
G = 4
NG = H // G
EPS = 1e-5
R = 512
DR = 32
DK = 3
LAG = 3
NVS = 16
QC = 512
N_LEAD = 32
N_LAST = 8


def _layernorm(x):
    m = jnp.mean(x, axis=-1, keepdims=True)
    xc = x - m
    v = jnp.mean(xc * xc, axis=-1, keepdims=True)
    return xc / jnp.sqrt(v + EPS)


def _gelu_tanh(x):
    c = 0.7978845608028654
    return 0.5 * x * (1.0 + jnp.tanh(c * (x + 0.044715 * (x * x * x))))


def _div(a, n):
    if isinstance(a, int):
        return a // n
    assert n & (n - 1) == 0
    return lax.shift_right_logical(a, n.bit_length() - 1)


def _mod(a, n):
    if isinstance(a, int):
        return a % n
    assert n & (n - 1) == 0
    return lax.bitwise_and(a, n - 1)


def _aligned(i, n):
    return i * n if isinstance(i, int) else pl.multiple_of(i * n, n)


def _wait_all(blk, sem):
    pltpu.make_async_copy(blk, blk, sem).wait()


def _loop(lo, hi, fn):
    def body(i, c):
        fn(i)
        return c
    lax.fori_loop(lo, hi, body, 0)


def _kernel(x_hbm, k_hbm, v_hbm, wq_hbm, wo_hbm, w3_hbm, w4_hbm, o_ref,
            x_buf, k_buf, v_buf, wq_buf, wo_buf, w3_buf, w4_buf,
            q_scr, s_scr, p_scr, acc_scr, out_scr, y_scr, h_scr, g_scr, xn_scr, coef_scr,
            sem_k, sem_v, sem_l, sem_m, *, sk, win):
    start = sk - win
    nc = win // R
    nd = R // DR
    nt = NG * nc
    d = x_buf.shape[-1]
    f = w3_buf.shape[0] * w3_buf.shape[1]
    wo_rows = G * DH
    n_rb = wo_rows // 8
    n_w3 = w3_buf.shape[1] // 16
    n_qc = H * DH // QC
    n_wq = (wq_buf.shape[1] // 8) * n_qc
    late_rows = N_LAST * 32
    s_x, s_wq, s_w3, s_w4, s_wo = (sem_m.at[i] for i in range(5))
    last_slot = (nt - 1) % NVS

    def k_desc(t, j):
        g, c = _div(t, nc), _mod(t, nc)
        return pltpu.make_async_copy(
            k_hbm.at[0, pl.ds(g * G, G), pl.ds(start + c * R + j * DR, DR), :],
            k_buf.at[c, :, pl.ds(j * DR, DR), :], sem_k.at[c])

    def v_desc(t, j):
        g, c, s = _div(t, nc), _mod(t, nc), _mod(t, NVS)
        return pltpu.make_async_copy(
            v_hbm.at[0, pl.ds(g * G, G), pl.ds(start + c * R + j * DR, DR), :],
            v_buf.at[s, :, pl.ds(j * DR, DR), :], sem_v.at[s])

    def v_last_desc(j, i):
        rr = R // 4
        return pltpu.make_async_copy(
            v_hbm.at[0, H - G + j, pl.ds(start + (nc - 1) * R + i * rr, rr), :],
            v_buf.at[last_slot, j, pl.ds(i * rr, rr), :], sem_l.at[j])

    def wq_desc(i):
        rows = pl.ds(_aligned(_div(i, n_qc), 8), 8)
        cols = pl.ds(_aligned(_mod(i, n_qc), QC), QC)
        return pltpu.make_async_copy(wq_hbm.at[:, rows, cols], wq_buf.at[:, rows, cols], s_wq)

    def wo_desc(g0, ng, i):
        idx = (pl.ds(g0, ng), pl.ds(_aligned(i, 8), 8), slice(None))
        return pltpu.make_async_copy(wo_hbm.at[idx], wo_buf.at[idx], s_wo)

    def wo_late_desc(i):
        idx = (0, pl.ds(i * 32, 32), slice(None))
        return pltpu.make_async_copy(wo_hbm.at[idx], wo_buf.at[idx], sem_l.at[G + i])

    def mlp_desc(src, dst, sem, i):
        idx = (slice(None), pl.ds(_aligned(i, 16), 16), slice(None))
        return pltpu.make_async_copy(src.at[idx], dst.at[idx], sem)

    x_cp = pltpu.make_async_copy(x_hbm, x_buf, s_x)
    x_cp.start(priority=0)

    _loop(0, N_LEAD, lambda i: mlp_desc(w3_hbm, w3_buf, s_w3, i).start(priority=1))

    n_q1 = N_LEAD // 2
    n_q0 = n_wq - n_q1
    a1 = n_w3 - N_LEAD
    a2 = a1 + n_q1
    n_lb = late_rows // 8
    a3 = a2 + n_lb
    a4 = a2 + n_rb
    n_b1 = n_q0 - a4

    def pairs(lo, hi, second):
        def fn(i):
            wq_desc(i).start(priority=0)
            second(i - lo).start(priority=1)
        _loop(lo, hi, fn)

    pairs(0, a1, lambda i: mlp_desc(w3_hbm, w3_buf, s_w3, N_LEAD + i))
    pairs(a1, a2, lambda i: wq_desc(n_q0 + i))

    x_cp.wait()
    xn_b = jnp.broadcast_to(_layernorm(x_buf[0].astype(jnp.float32)), (8, d)).astype(jnp.bfloat16)
    xn_scr[...] = xn_b
    y_scr[...] = _layernorm(xn_b.astype(jnp.float32)).astype(jnp.bfloat16)
    acc_scr[...] = jnp.zeros_like(acc_scr)
    out_scr[...] = jnp.zeros_like(out_scr)

    pairs(a2, a3, lambda i: wo_desc(1, 3, i))
    pairs(a3, a4, lambda i: wo_desc(0, 4, n_lb + i))
    pairs(a4, n_q0, lambda i: wo_desc(4, 4, i))

    _wait_all(w3_buf, s_w3)
    hmid = lax.dot_general(y_scr[...], w3_buf[...].reshape(f, d), (((1,), (1,)), ((), ())),
                           preferred_element_type=jnp.float32)
    h_scr[...] = _gelu_tanh(hmid).astype(jnp.bfloat16)

    n_b = n_rb - n_b1
    assert n_b <= LAG * nd and DK == LAG

    def pair_k_wo(i):
        k_desc(_div(i, nd), _mod(i, nd)).start(priority=0)
        wo_desc(4, 4, n_b1 + i).start(priority=1)
    _loop(0, n_b, pair_k_wo)
    _loop(n_b, LAG * nd, lambda i: k_desc(_div(i, nd), _mod(i, nd)).start(priority=0))

    _wait_all(wq_buf, s_wq)
    q_all = jnp.dot(xn_scr[...], wq_buf[...].reshape(d, H * DH),
                    preferred_element_type=jnp.float32).astype(jnp.bfloat16)
    for h in range(H):
        q_scr[h] = q_all[:, h * DH:(h + 1) * DH]

    scale = DH ** -0.5
    row = lax.broadcasted_iota(jnp.int32, (8, R), 0)
    row_d = lax.broadcasted_iota(jnp.int32, (8, DH), 0)

    def qk(t):
        g, c = _div(t, nc), _mod(t, nc)
        s = None
        for j in range(G):
            sj = lax.dot_general(q_scr[g * G + j], k_buf[c, j], (((1,), (1,)), ((), ())),
                                 preferred_element_type=jnp.float32)
            s = sj if s is None else jnp.where(row == j, sj, s)
        s_scr[c] = s

    def softmax():
        s = s_scr[...]
        m = jnp.max(jnp.max(s, axis=0), axis=-1, keepdims=True)
        p = jnp.exp((s - m[None]) * scale)
        l = jnp.sum(jnp.sum(p, axis=0), axis=-1, keepdims=True)
        p_scr[...] = (p * (1.0 / l)[None]).astype(jnp.bfloat16)

    def pv(u):
        p = p_scr[_mod(u, nc)]
        o = None
        for j in range(G):
            oj = jnp.dot(p, v_buf[_mod(u, NVS), j], preferred_element_type=jnp.float32)
            o = oj if o is None else jnp.where(row_d == j, oj, o)
        acc_scr[...] += o

    def finalize(g):
        o = acc_scr[...]
        acc_scr[...] = jnp.zeros_like(acc_scr)
        lhs = jnp.concatenate([jnp.where(row_d == j, o, 0.0) for j in range(G)],
                              axis=1).astype(jnp.bfloat16)

        @pl.when(g > 0)
        def _():
            out_scr[...] += jnp.dot(lhs, wo_buf[g], preferred_element_type=jnp.float32)

        @pl.when(g == 0)
        def _():
            out_scr[...] += jnp.dot(lhs[:, late_rows:], wo_buf[0, pl.ds(late_rows, wo_rows - late_rows), :],
                                    preferred_element_type=jnp.float32)
            eye = (lax.broadcasted_iota(jnp.int32, (DH, DH), 0)
                   == lax.broadcasted_iota(jnp.int32, (DH, DH), 1)).astype(jnp.bfloat16)
            ob = o.astype(jnp.bfloat16)
            for j in range(late_rows // DH):
                rows = jnp.broadcast_to(ob[j:j + 1, :], (DH, DH))
                coef_scr[pl.ds(j * DH, DH), :] = lax.dot_general(
                    eye, rows, (((1,), (1,)), ((), ())), preferred_element_type=jnp.float32)

    n_steps = nt + nc
    assert n_w3 <= LAG * nd and nd == 4 * G and late_rows % DH == 0

    w4_per = -(-n_w3 // (LAG - 1))

    def step(t, carry):
        tk = t + DK

        @pl.when(tk < nt)
        def _():
            for j in range(nd):
                k_desc(tk, j).start(priority=0)
                v_desc(tk - LAG, j).start(priority=1)

        for i in range(LAG):
            @pl.when(tk == nt + i)
            def _(i=i):
                lo = min(i * w4_per, n_w3)
                hi = min((i + 1) * w4_per, n_w3)
                for j in range(max(nd, hi - lo)):
                    if lo + j < hi:
                        mlp_desc(w4_hbm, w4_buf, s_w4, lo + j).start(priority=0)
                    if j < nd:
                        if i < LAG - 1:
                            v_desc(nt - LAG + i, j).start(priority=1)
                        else:
                            v_last_desc(j // 4, j % 4).start(priority=1)
                if i == LAG - 1:
                    for ii in range(N_LAST):
                        wo_late_desc(ii).start(priority=1)

        @pl.when(t < nt)
        def _():
            _wait_all(k_buf.at[_mod(t, nc)], sem_k.at[_mod(t, nc)])
            qk(t)

        @pl.when(t == n_steps - 2)
        def _():
            _wait_all(w4_buf, s_w4)
            h2 = jnp.dot(h_scr[...], w4_buf[...].reshape(f, d), preferred_element_type=jnp.float32)
            b = xn_scr[...].astype(jnp.float32) + h2
            g_scr[...] = b * jax.nn.sigmoid(b)

        @pl.when(t >= nc)
        def _():
            s = _mod(t - nc, NVS)
            _wait_all(v_buf.at[s], sem_v.at[s])
            pv(t - nc)

        @pl.when(_mod(t, nc) == nc - 1)
        def _():
            @pl.when(t == 2 * nc - 1)
            def _():
                _wait_all(wo_buf.at[pl.ds(1, NG - 1)], s_wo)
                _wait_all(wo_buf.at[0, pl.ds(late_rows, wo_rows - late_rows), :], s_wo)

            @pl.when(t >= nc)
            def _():
                finalize(_div(t - nc, nc))

            @pl.when(t < nt)
            def _():
                softmax()
        return carry

    lax.fori_loop(0, n_steps - 1, step, 0)

    def last_op(lhs, j):
        return jnp.dot(lhs, wo_buf[NG - 1, pl.ds(j * DH, DH), :], preferred_element_type=jnp.float32)

    out_acc = out_scr[...]
    prev = None
    for j in range(G):
        _wait_all(v_buf.at[last_slot, j], sem_l.at[j])
        oj = jnp.dot(p_scr[nc - 1], v_buf[last_slot, j], preferred_element_type=jnp.float32)
        if prev is not None:
            out_acc = out_acc + last_op(prev, j - 1)
        prev = jnp.where(row_d == j, acc_scr[...] + oj, 0.0).astype(jnp.bfloat16)
    out_acc = out_acc + last_op(prev, G - 1)
    for i in range(N_LAST):
        rows = pl.ds(i * 32, 32)
        _wait_all(wo_buf.at[0, rows, :], sem_l.at[G + i])
        w = wo_buf[0, rows, :].astype(jnp.float32)
        for k in range(4):
            c = coef_scr[pl.ds(i * 32 + k * 8, 8), :]
            out_acc = out_acc + w[k * 8:(k + 1) * 8, :] * jnp.concatenate([c] * (d // DH), axis=1)
    attn = jnp.sum(out_acc, axis=0, keepdims=True)
    out = x_buf[0].astype(jnp.float32) + attn * g_scr[0:1, :]
    o_ref[0] = out.astype(o_ref.dtype)


@jax.jit
def pallas_recurrent_scan__sliding_block_cached__mixer_s_mlp__decode_kernel(
    A_x: jax.Array,
    A_k_cache: jax.Array,
    A_v_cache: jax.Array,
    A_wq: jax.Array,
    A_wo: jax.Array,
    B_x: jax.Array,
    B_w1: jax.Array,
    B_w2: jax.Array,
    B_w3: jax.Array,
    B_w4: jax.Array,
):
    _, _, d = A_x.shape
    sk = A_k_cache.shape[2]
    win = min(4096, max(256, sk // 4))
    f = B_w3.shape[1]
    bf = jnp.bfloat16
    f32 = jnp.float32
    nc = win // R
    any_spec = pl.BlockSpec(memory_space=pl.ANY)
    return pl.pallas_call(
        functools.partial(_kernel, sk=sk, win=win),
        out_shape=jax.ShapeDtypeStruct(A_x.shape, A_x.dtype),
        in_specs=[any_spec] * 7,
        out_specs=pl.BlockSpec(memory_space=pltpu.VMEM),
        scratch_shapes=[
            pltpu.VMEM(A_x.shape, bf),
            pltpu.VMEM((nc, G, R, DH), bf),
            pltpu.VMEM((NVS, G, R, DH), bf),
            pltpu.VMEM((4, d // 4, H * DH), bf),
            pltpu.VMEM((NG, G * DH, d), bf),
            pltpu.VMEM((2, f // 2, d), bf),
            pltpu.VMEM((2, f // 2, d), bf),
            pltpu.VMEM((H, 8, DH), bf),
            pltpu.VMEM((nc, 8, R), f32),
            pltpu.VMEM((nc, 8, R), bf),
            pltpu.VMEM((8, DH), f32),
            pltpu.VMEM((8, d), f32),
            pltpu.VMEM((8, d), bf),
            pltpu.VMEM((8, f), bf),
            pltpu.VMEM((8, d), f32),
            pltpu.VMEM((8, d), bf),
            pltpu.VMEM((N_LAST * 32, DH), f32),
            pltpu.SemaphoreType.DMA((nc,)),
            pltpu.SemaphoreType.DMA((NVS,)),
            pltpu.SemaphoreType.DMA((G + N_LAST,)),
            pltpu.SemaphoreType.DMA((5,)),
        ],
        compiler_params=pltpu.CompilerParams(
            vmem_limit_bytes=64 * 1024 * 1024,
            disable_bounds_checks=True,
            disable_semaphore_checks=True,
        ),
    )(A_x, A_k_cache, A_v_cache,
      A_wq.reshape(4, d // 4, H * DH), A_wo.reshape(NG, G * DH, d),
      B_w3.T.reshape(2, f // 2, d), B_w4.reshape(2, f // 2, d))
```
